```python
import jax
import jax.numpy as jnp

def _softmax(x, axis=-1):
    return jax.nn.softmax(x, axis=axis)
def _gelu(x):
    return jax.nn.gelu(x, approximate=True)
def _silu(x):
    return jax.nn.silu(x)
def _sigmoid(x):
    return jax.nn.sigmoid(x)
def _layernorm(x, axis=-1, eps=1e-5):
    m = jnp.mean(x, axis=axis, keepdims=True)
    v = jnp.var(x, axis=axis, keepdims=True)
    return (x - m) / jnp.sqrt(v + eps)
def _scatter_add(tgt, idx, src, axis=0):
    return tgt.at[idx].add(src)
def _segment_sum(src, seg, n):
    return jax.ops.segment_sum(src, seg, n)
class _Rng:
    def __init__(self, key):
        self._k = key
    def _next(self):
        self._k, sub = jax.random.split(self._k)
        return sub
    def normal(self, shape):
        return jax.random.normal(self._next(), shape, dtype=jnp.bfloat16)
    def randint(self, lo, hi, shape):
        return jax.random.randint(self._next(), shape, lo, hi, dtype=jnp.int32)
    def uniform(self, shape, lo=0.0, hi=1.0):
        return jax.random.uniform(self._next(), shape, jnp.bfloat16, lo, hi)
    def permutation(self, n):
        return jax.random.permutation(self._next(), n)


kernel_name = 'recurrent_scan__compressed_kv_cla__moe_arch_mod__decode'

def setup_inputs():
    _rng = _Rng(jax.random.key(int.from_bytes(__import__("os").urandom(4), "little")))
    _w = (lambda a: (lambda t: t.astype(jnp.bfloat16) if jnp.issubdtype(t.dtype, jnp.floating) else t)(jnp.asarray(a)))
    def _A_setup():
        B, H, Sq, Sk, D, M = 4, 32, 1, 4096, 128, 576
        Dc = 4 * D
        return {
            "x": _w((lambda *s: _rng.normal(s) * 0.05)(B, Sq, M)),
            "c_kv": _w((lambda *s: _rng.normal(s) * 0.05)(B, Sk, Dc)),
            "w_q": _w((lambda *s: _rng.normal(s) * 0.05)(M, H, D) * (M ** -0.5)),
            "w_uk": _w((lambda *s: _rng.normal(s) * 0.05)(Dc, H, D) * (Dc ** -0.5)),
            "w_uv": _w((lambda *s: _rng.normal(s) * 0.05)(Dc, H, D) * (Dc ** -0.5)),
            "w_o": _w((lambda *s: _rng.normal(s) * 0.05)(H, D, M) * ((H * D) ** -0.5)),
        }
    _A_in = _A_setup()

    def _B_setup():
        B, S, D, F, C = 4, 1, 576, 4608, 1
        return {
            "x": _w((lambda *s: _rng.normal(s) * 0.05)(B, S, D)),
            "w_r": _w((lambda *s: _rng.normal(s) * 0.05)(D)),
            "w_gate": _w((lambda *s: _rng.normal(s) * 0.05)(D, F)),
            "w_up": _w((lambda *s: _rng.normal(s) * 0.05)(D, F)),
            "w_down": _w((lambda *s: _rng.normal(s) * 0.05)(F, D)),
        }
    _B_in = _B_setup()

    return {
        "A_x": _A_in["x"],
        "A_c_kv": _A_in["c_kv"],
        "A_w_q": _A_in["w_q"],
        "A_w_uk": _A_in["w_uk"],
        "A_w_uv": _A_in["w_uv"],
        "A_w_o": _A_in["w_o"],
        "B_x": _B_in["x"],
        "B_w_r": _B_in["w_r"],
        "B_w_gate": _B_in["w_gate"],
        "B_w_up": _B_in["w_up"],
        "B_w_down": _B_in["w_down"],
    }

def reference(A_x, A_c_kv, A_w_q, A_w_uk, A_w_uv, A_w_o, B_x, B_w_r, B_w_gate, B_w_up, B_w_down):
    def _A_ref(x, c_kv, w_q, w_uk, w_uv, w_o):
        B, Sq, M = x.shape[0], x.shape[1], x.shape[2]
        Sk = c_kv.shape[1]
        H, D = w_q.shape[1], w_q.shape[2]
        q = jnp.einsum("bqm,mhd->bhqd", x, w_q)
        k = jnp.einsum("bkc,chd->bhkd", c_kv, w_uk)
        v = jnp.einsum("bkc,chd->bhkd", c_kv, w_uv)
        scores = jnp.einsum("bhqd,bhkd->bhqk", q, k) * (D ** -0.5)
        off = Sk - Sq
        qi = jnp.arange(Sq)[:, None]
        kj = jnp.arange(Sk)[None, :]
        cmask = kj <= (qi + off)
        scores = jnp.where(cmask[None, None], scores, -1e9)
        p = _softmax(scores, axis=-1)
        ctx = jnp.einsum("bhqk,bhkd->bhqd", p, v)
        return jnp.einsum("bhqd,hdm->bqm", ctx, w_o)

    def _B_ref(x, w_r, w_gate, w_up, w_down):
        B, S, D = x.shape
        C = 1
        r = x @ w_r
        idx = jnp.argsort(-r, axis=-1)[:, :C]
        idx_e = jnp.repeat(idx.reshape(B, C, 1), D, axis=2)
        x_sel = jnp.take_along_axis(x, idx_e, axis=1)
        g = _silu(x_sel @ w_gate)
        u = x_sel @ w_up
        y = (g * u) @ w_down
        r_sel = _sigmoid(jnp.take_along_axis(r, idx, axis=1))
        y = y * r_sel.reshape(B, C, 1)
        b_off = (jnp.arange(B) * S).reshape(B, 1)
        flat_idx = (idx + b_off).reshape(B * C)
        zero = (x * 0.0).reshape(B * S, D)
        upd = _scatter_add(zero, flat_idx, y.reshape(B * C, D), axis=0)
        return x + upd.reshape(B, S, D)

    x = A_x
    xn = _layernorm(x, axis=-1)
    s = _A_ref(xn, A_c_kv, A_w_q, A_w_uk, A_w_uv, A_w_o)
    g = _silu(_B_ref(xn, B_w_r, B_w_gate, B_w_up, B_w_down))
    return x + s * g
```

```python
import jax
import jax.numpy as jnp
from jax import lax
import jax.experimental.pallas as pl
import jax.experimental.pallas.tpu as pltpu

_F32 = jnp.float32
_BF16 = jnp.bfloat16
_LANES = 128
_TILE_ROWS = 8
_SLAB = 32
_HG = 16

_WQ, _WUK, _CKV, _WUV, _WG, _WU, _WD, _WO = range(8)

_PIECE = 2
_COLUMN = 128
_PRIORITIES = (0, 1, 1, 1, 1)
_LAG = 6
_WO_EARLY = 0
_WO_GROUP = 24
_WO_WHOLE = 16
_WO_LAST = (16, 12, 8, 8, 4)
_DOWN_STEP = 8
_STEP = 11
_QK_STEP = 5
_PV_STEP = 5
_COPY_ONLY = False
_QUEUE = 80


def _dot(a, b):
    return jnp.dot(a, b, preferred_element_type=_F32)


def _dot_nt(a, b):
    return lax.dot_general(a, b, (((1,), (1,)), ((), ())), preferred_element_type=_F32)


def _iota(shape, axis):
    return lax.broadcasted_iota(jnp.int32, shape, axis)


def _pad_rows(v, rows=8):
    return jnp.concatenate([v, jnp.zeros((rows - v.shape[0], v.shape[1]), v.dtype)], axis=0)


def _stream_order(sizes):
    def columns(operand, first=0, last=None):
        return [(operand, s) for s in range(0, sizes[operand], _COLUMN)][first:last]

    def rows(cols, parts):
        height = _COLUMN // parts
        offsets = sorted(range(0, _COLUMN, height), key=lambda s: s & -s, reverse=True)
        offsets = offsets[-1:] + offsets[:-1]
        return [
            (operand, s + offset + row)
            for row in range(0, height, _PIECE)
            for offset in offsets
            for operand, s in cols
            if s + offset + row < sizes[operand]
        ]

    return (
        rows(columns(_WQ) + columns(_WUK) + columns(_WUV), 1)
        + rows(columns(_CKV), 1)
        + rows(columns(_WG) + columns(_WU), 1)
        + rows(columns(_WO, 0, _WO_EARLY) + columns(_WD), 2)
        + rows(columns(_WO, _WO_EARLY), 2)
    )


class _Stream:
    def __init__(self, order, sources, bases, buf, sems):
        self.sources, self.bases, self.buf, self.sems = sources, bases, buf, sems
        priority = [_PRIORITIES[i % len(_PRIORITIES)] for i in range(len(order))]
        high = [i for i, p in enumerate(priority) if p == 0]
        place = {i: i for i in range(len(order))}
        for k, i in enumerate(high):
            place[i] = high[k + _LAG] - 0.5 if k + _LAG < len(high) else len(order) + k
        self.todo = [order[i] + (priority[i],) for i in sorted(place, key=place.get)]
        self.ready = {g: i + _QUEUE for i, (g, *_) in enumerate(self.todo)}
        self.done = 0

    def _copy(self, g, operand, start):
        return pltpu.make_async_copy(
            self.sources[operand].at[pl.ds(start, _PIECE)],
            self.buf.at[pl.ds(self.bases[operand] + start, _PIECE)],
            self.sems.at[g],
        )

    def advance(self, count=None):
        count = _STEP if count is None else count
        for *copy, priority in self.todo[self.done:self.done + count]:
            self._copy(*copy).start(priority=priority)
        self.done = min(self.done + count, len(self.todo))

    def wait(self, g):
        self.advance(max(self.ready[g] - self.done, 0))
        copies = [c[:3] for c in self.todo if c[0] == g]
        operand = copies[0][1]
        size = self.sources[operand].shape[0]
        if len(copies) * _PIECE == size:
            filled = self.buf.at[pl.ds(self.bases[operand], size)]
            pltpu.make_async_copy(filled, filled, self.sems.at[g]).wait()
        else:
            for copy in copies:
                self._copy(*copy).wait()


def _kernel(
    x_hbm, wr_hbm, wq_hbm, wuk_hbm, ckv_hbm, wuv_hbm, wg_hbm, wu_hbm, wd_hbm, wo_hbm,
    out_hbm,
    buf, x_v, wr_v, out_v, lhs_v, ctx_v, rows_v, sems, small_sems,
    *, heads, keys, hidden_dim,
):
    B, M = x_v.shape
    D = _LANES
    Dc = wuk_hbm.shape[0]
    n_groups = heads // _HG
    rows = B * _HG
    per_tile = _LANES // _HG
    n_expand = _LANES // per_tile

    sources = [wq_hbm, wuk_hbm, ckv_hbm, wuv_hbm, wg_hbm, wu_hbm, wd_hbm, wo_hbm]
    bases = [0]
    for src in sources:
        bases.append(bases[-1] + src.shape[0])
    q0, uk0, kv0, uv0, g0, u0, d0, o0, expand0 = bases

    head_slabs, tile_slabs = M // _SLAB, _LANES // _SLAB
    lane_tiles = [(t, min(tile_slabs, head_slabs - t)) for t in range(0, head_slabs, tile_slabs)]
    wo_tiles = [
        (h, i, h * head_slabs + t, n) for h in range(heads) for i, (t, n) in enumerate(lane_tiles)
    ]
    last_tiles = [
        next(t for t in wo_tiles if t[:2] == (k * heads // _WO_WHOLE, (_WO_WHOLE - 1 - k) // 4 % 4))
        for k in range(_WO_WHOLE)
    ]
    last = [start + k for _, _, start, n in last_tiles for k in range(0, n, _PIECE)]
    order = _stream_order([src.shape[0] for src in sources])
    order = [p for p in order if p[0] != _WO or p[1] not in last] + [(_WO, s) for s in last]
    place = {s: i for i, (operand, s) in enumerate(order) if operand == _WO}
    wo_tiles.sort(key=lambda t: max(place[t[2] + k] for k in range(0, t[3], _PIECE)))
    cuts = [len(wo_tiles) - sum(_WO_LAST[i:]) for i in range(len(_WO_LAST) + 1)]
    cuts = list(range(cuts[0] % _WO_GROUP or _WO_GROUP, cuts[0], _WO_GROUP)) + cuts
    wo_groups = [wo_tiles[a:b] for a, b in zip([0] + cuts[:-1], cuts)]
    group_of = {
        start + k: g
        for g, tiles in enumerate(wo_groups, _WO)
        for _, _, start, n in tiles
        for k in range(0, n, _PIECE)
    }
    stream = _Stream(
        [(group_of[s] if operand == _WO else operand, operand, s) for operand, s in order],
        sources, bases, buf, sems,
    )

    def flat(start, n):
        return buf[start:start + n].reshape(n * _SLAB, _LANES)

    def head_group(base, row0, n, g):
        return buf[base + row0:base + row0 + n, g * _HG:(g + 1) * _HG, :].reshape(n * _HG, D)

    per_slab = _SLAB // _TILE_ROWS

    def cache_tile(k0, n, j):
        first = kv0 + k0 // _TILE_ROWS
        tile = slice(j * _TILE_ROWS, (j + 1) * _TILE_ROWS)
        return buf[first:first + n // _TILE_ROWS, tile, :].reshape(n, _LANES)

    def column_tiles(base):
        per_band = hidden_dim // _LANES // per_slab
        for c in range(per_band):
            slabs = [buf[base + i * per_band + c] for i in range(M // _TILE_ROWS)]
            for r in range(0, _SLAB, _TILE_ROWS):
                yield jnp.concatenate([slab[r:r + _TILE_ROWS] for slab in slabs], axis=0)

    def expand(t):
        return flat(expand0 + t * _LANES // _SLAB, _LANES // _SLAB)

    x_cp = pltpu.make_async_copy(x_hbm, x_v, small_sems.at[0])
    wr_cp = pltpu.make_async_copy(wr_hbm, wr_v, small_sems.at[1])
    stream.advance(8)
    x_cp.start()
    wr_cp.start()
    stream.advance(_QUEUE)

    if _COPY_ONLY:
        x_cp.wait()
        wr_cp.wait()
        stream.advance(10000)
        for g in sorted(stream.ready):
            stream.wait(g)
        out_v[...] = x_v[...]
        out_cp = pltpu.make_async_copy(out_v, out_hbm, small_sems.at[0])
        out_cp.start()
        out_cp.wait()
        return
    square = (_LANES, _LANES)
    for t in range(n_expand):
        e = _iota(square, 1) // _HG + t * per_tile == _iota(square, 0)
        first = expand0 + t * _LANES // _SLAB
        buf[first:first + _LANES // _SLAB] = e.astype(_BF16).reshape(-1, _SLAB, _LANES)
        if t % 4 == 3:
            stream.advance()
    own_head = _iota((rows, _LANES), 1) % _HG == _iota((rows, _LANES), 0) % _HG

    x_cp.wait()
    wr_cp.wait()
    x = _pad_rows(x_v[...].astype(_F32))
    xc = x - jnp.mean(x, axis=-1, keepdims=True)
    xn_lo = (xc / jnp.sqrt(jnp.mean(xc * xc, axis=-1, keepdims=True) + 1e-5)).astype(_BF16)
    xn = xn_lo.astype(_F32)
    wr = wr_v[...].astype(_F32).reshape(1, M)
    route = jax.nn.sigmoid(jnp.sum(xn * wr, axis=-1, keepdims=True))

    for t in range(M // per_tile):
        m0 = t // n_expand * _LANES
        n = min(_LANES, M - m0)
        rep = _dot(xn_lo[:, m0:m0 + n], expand(t % n_expand)[:n])
        rep = jnp.concatenate(
            [jnp.broadcast_to(rep[b:b + 1], (_HG, _LANES)) for b in range(B)], axis=0
        )
        lhs_v[t] = jnp.where(own_head, rep, 0.0).astype(_BF16)
        if t % 3 == 2:
            stream.advance()
    stream.wait(_WQ)
    q = [jnp.zeros((rows, D), _F32) for _ in range(n_groups)]
    for t in range(M // per_tile):
        lhs = lhs_v[t]
        for g in range(n_groups):
            q[g] = q[g] + _dot(lhs, head_group(q0, t * per_tile, per_tile, g))
        if t % 6 == 5:
            stream.advance()

    stream.wait(_WUK)
    q_lat = []
    for g in range(n_groups):
        qg = q[g].astype(_BF16)
        tiles = []
        for c0 in range(0, Dc, _LANES):
            acc = jnp.zeros((rows, _LANES), _F32)
            for t in range(n_expand):
                full = _dot_nt(qg, head_group(uk0, c0 + t * per_tile, per_tile, g))
                acc = acc + _dot_nt(jnp.where(own_head, full, 0.0).astype(_BF16), expand(t))
                if t % 4 == 3:
                    stream.advance()
            tiles.append(acc.astype(_BF16))
        q_lat.append(tiles)

    qk_keys, pv_keys = 512, 1024
    lat_tiles = range(Dc // _LANES)

    def scores(b):
        qb = [
            jnp.concatenate([q_lat[g][j][b * _HG:(b + 1) * _HG] for g in range(n_groups)], axis=0)
            for j in lat_tiles
        ]
        chunks = []
        for k0 in range(b * keys, (b + 1) * keys, qk_keys):
            parts = []
            for j in lat_tiles:
                parts.append(_dot_nt(qb[j], cache_tile(k0, qk_keys, j)))
                if j % 2:
                    stream.advance(_QK_STEP)
            chunks.append(sum(parts[1:], parts[0]))
        return jnp.concatenate(chunks, axis=1) * (D ** -0.5)

    def attend(b, s):
        p = jnp.exp(s - jnp.max(s, axis=-1, keepdims=True))
        denom = jnp.sum(p, axis=-1, keepdims=True)
        p = p.astype(_BF16)
        acc = [jnp.zeros((heads, _LANES), _F32) for _ in lat_tiles]
        for k0 in range(0, keys, pv_keys):
            for j in lat_tiles:
                acc[j] = acc[j] + _dot(p[:, k0:k0 + pv_keys], cache_tile(b * keys + k0, pv_keys, j))
                stream.advance(_PV_STEP)
        return [(a / denom).astype(_BF16) for a in acc]

    stream.wait(_CKV)
    lat = []
    s = scores(0)
    for b in range(B):
        ahead = scores(b + 1) if b + 1 < B else None
        lat.append(attend(b, s))
        s = ahead

    stream.wait(_WUV)
    for g in range(n_groups):
        ctx = jnp.zeros((rows, D), _F32)
        for j in range(Dc // _LANES):
            lg = jnp.concatenate([lb[j][g * _HG:(g + 1) * _HG] for lb in lat], axis=0)
            for t in range(n_expand):
                lhs = jnp.where(own_head, _dot(lg, expand(t)), 0.0).astype(_BF16)
                ctx = ctx + _dot(lhs, head_group(uv0, j * _LANES + t * per_tile, per_tile, g))
                if t % 8 == 7:
                    stream.advance()
        ctx_v[:, g * _HG:(g + 1) * _HG, :] = ctx.reshape(B, _HG, D)
    for h in range(heads):
        rows_v[h] = _pad_rows(ctx_v[:, h, :], 2 * _TILE_ROWS).astype(_BF16)

    def project(base):
        tiles = []
        for j, w in enumerate(column_tiles(base)):
            tiles.append(_dot(xn_lo, w))
            if j % 6 == 5:
                stream.advance()
        return tiles

    stream.wait(_WG)
    gate = [jax.nn.silu(v) for v in project(g0)]
    stream.wait(_WU)
    hidden = [(a * v).astype(_BF16) for a, v in zip(gate, project(u0))]

    s = [jnp.zeros((x.shape[0], n * _SLAB), _F32) for _, n in lane_tiles]

    stream.wait(_WD)
    y = jnp.zeros(x.shape, _F32)
    for j, w in enumerate(column_tiles(d0)):
        y = y + _dot_nt(hidden[j], w)
        if j % 3 == 2:
            stream.advance(_DOWN_STEP)
    mixed = jax.nn.silu(xn + (xn * 0.0 + y * route))
    for g, tiles in enumerate(wo_groups, _WO):
        stream.wait(g)
        for h, i, start, n in tiles:
            s[i] = s[i] + _dot_nt(rows_v[h][:_TILE_ROWS], flat(o0 + start, n))

    out = x + jnp.concatenate(s, axis=1) * mixed
    out_v[...] = out.astype(out_v.dtype)[:B]
    out_cp = pltpu.make_async_copy(out_v, out_hbm, small_sems.at[0])
    out_cp.start()
    out_cp.wait()


def _slabs(w):
    r, c = w.shape
    w = w.reshape(r // _TILE_ROWS, _TILE_ROWS, c // _LANES, _LANES)
    return w.transpose(0, 2, 1, 3).reshape(-1, _SLAB, _LANES)


@jax.jit
def pallas_recurrent_scan__compressed_kv_cla__moe_arch_mod__decode_kernel(
    A_x: jax.Array,
    A_c_kv: jax.Array,
    A_w_q: jax.Array,
    A_w_uk: jax.Array,
    A_w_uv: jax.Array,
    A_w_o: jax.Array,
    B_x: jax.Array,
    B_w_r: jax.Array,
    B_w_gate: jax.Array,
    B_w_up: jax.Array,
    B_w_down: jax.Array,
):
    del B_x
    B, Sq, M = A_x.shape
    _, Sk, Dc = A_c_kv.shape
    _, H, D = A_w_q.shape
    assert Sq == 1 and H == _SLAB and D == _LANES

    x = A_x.reshape(B, M)
    streamed = [
        A_w_q,
        A_w_uk,
        _slabs(A_c_kv.reshape(B * Sk, Dc)),
        A_w_uv,
        _slabs(B_w_gate),
        _slabs(B_w_up),
        _slabs(B_w_down.T),
        jnp.transpose(A_w_o, (0, 2, 1)).reshape(-1, _SLAB, _LANES),
    ]
    n_slabs = sum(w.shape[0] for w in streamed) + _HG * _LANES // _SLAB

    def kernel(*refs):
        _kernel(*refs, heads=H, keys=Sk, hidden_dim=B_w_gate.shape[1])

    hbm = pl.BlockSpec(memory_space=pltpu.HBM)
    out = pl.pallas_call(
        kernel,
        out_shape=jax.ShapeDtypeStruct((B, M), A_x.dtype),
        in_specs=[hbm] * (2 + len(streamed)),
        out_specs=hbm,
        scratch_shapes=[
            pltpu.VMEM((n_slabs, _SLAB, _LANES), _BF16),
            pltpu.VMEM(x.shape, x.dtype),
            pltpu.VMEM(B_w_r.shape, B_w_r.dtype),
            pltpu.VMEM(x.shape, x.dtype),
            pltpu.VMEM((M * _HG // D, B * _HG, D), _BF16),
            pltpu.VMEM((B, H, D), _F32),
            pltpu.VMEM((H, 2 * _TILE_ROWS, D), _BF16),
            pltpu.SemaphoreType.DMA((len(streamed) + 16,)),
            pltpu.SemaphoreType.DMA((2,)),
        ],
        compiler_params=pltpu.CompilerParams(
            vmem_limit_bytes=96 * 1024 * 1024, disable_semaphore_checks=True
        ),
    )(x, B_w_r, *streamed)
    return out.reshape(B, Sq, M)
```

```python
import jax
import jax.numpy as jnp
from jax import lax
import jax.experimental.pallas as pl
import jax.experimental.pallas.tpu as pltpu

_F32 = jnp.float32
_BF16 = jnp.bfloat16
_LANES = 128
_TILE_ROWS = 8
_SLAB = 32
_HG = 16

_WQ, _WUK, _CKV, _WUV, _WG, _WU, _WD, _WO = range(8)

_PIECE = 2
_PHASES = (
    ((_WUV, _WUK, _WQ), 128),
    ((_CKV,), 128),
    ((_WU, _WG), 128),
    ((_WD,), 64),
    ((_WO,), 64),
)
_HIGH_EVERY = 5
_OVERTAKE = 30
_LOW_AT_END = 24
_QUEUE = 80
_WO_GROUP = 24
_WO_LAST = (12, 12, 8, 4, 4)
_STEP, _ATTENTION_STEP, _DOWN_STEP = 11, 5, 8


def _dot(a, b):
    return jnp.dot(a, b, preferred_element_type=_F32)


def _dot_nt(a, b):
    return lax.dot_general(a, b, (((1,), (1,)), ((), ())), preferred_element_type=_F32)


def _iota(shape, axis):
    return lax.broadcasted_iota(jnp.int32, shape, axis)


def _pad_rows(v, rows=_TILE_ROWS):
    return jnp.concatenate([v, jnp.zeros((rows - v.shape[0], v.shape[1]), v.dtype)], axis=0)


def _stream_order(sizes):
    order = []
    for operands, stride in _PHASES:
        pieces = [(o, s) for o in operands for s in range(0, sizes[o], _PIECE)]
        for row in range(stride // _PIECE):
            order += pieces[row::stride // _PIECE]
    return order


class _Stream:
    def __init__(self, order, sources, bases, buf, sems):
        self.sources, self.bases, self.buf, self.sems = sources, bases, buf, sems
        is_high = [
            i % _HIGH_EVERY == 0 and i < len(order) - _LOW_AT_END for i in range(len(order))
        ]
        queued = sorted(range(len(order)), key=lambda i: i + is_high[i] * (_OVERTAKE - 0.5))
        self.todo = [order[i] + (0 if is_high[i] else 1,) for i in queued]
        self.ready = {g: i + _QUEUE for i, (g, *_) in enumerate(self.todo)}
        self.done = 0

    def _copy(self, g, operand, start):
        return pltpu.make_async_copy(
            self.sources[operand].at[pl.ds(start, _PIECE)],
            self.buf.at[pl.ds(self.bases[operand] + start, _PIECE)],
            self.sems.at[g],
        )

    def advance(self, count=_STEP):
        for *copy, priority in self.todo[self.done:self.done + count]:
            self._copy(*copy).start(priority=priority)
        self.done = min(self.done + count, len(self.todo))

    def wait(self, g):
        self.advance(max(self.ready[g] - self.done, 0))
        copies = [c[:3] for c in self.todo if c[0] == g]
        operand = copies[0][1]
        size = self.sources[operand].shape[0]
        if len(copies) * _PIECE == size:
            filled = self.buf.at[pl.ds(self.bases[operand], size)]
            pltpu.make_async_copy(filled, filled, self.sems.at[g]).wait()
        else:
            for copy in copies:
                self._copy(*copy).wait()


def _kernel(
    x_hbm, wr_hbm, wq_hbm, wuk_hbm, ckv_hbm, wuv_hbm, wg_hbm, wu_hbm, wd_hbm, wo_hbm,
    out_hbm,
    buf, x_v, wr_v, out_v, lhs_v, ctx_v, rows_v, sems, small_sems,
    *, heads, keys, hidden_dim,
):
    B, M = x_v.shape
    D = _LANES
    Dc = wuk_hbm.shape[0]
    n_groups = heads // _HG
    rows = B * _HG
    per_tile = _LANES // _HG
    n_expand = _LANES // per_tile

    sources = [wq_hbm, wuk_hbm, ckv_hbm, wuv_hbm, wg_hbm, wu_hbm, wd_hbm, wo_hbm]
    bases = [0]
    for src in sources:
        bases.append(bases[-1] + src.shape[0])
    q0, uk0, kv0, uv0, g0, u0, d0, o0, expand0 = bases

    head_slabs, tile_slabs = M // _SLAB, _LANES // _SLAB
    lane_tiles = [(t, min(tile_slabs, head_slabs - t)) for t in range(0, head_slabs, tile_slabs)]
    wo_tiles = [
        (h, i, h * head_slabs + t, n) for h in range(heads) for i, (t, n) in enumerate(lane_tiles)
    ]
    n_final = sum(_WO_LAST[-2:])
    whole = [t for t in wo_tiles if t[1] == 1][:_WO_LAST[-3]]
    whole += [t for t in wo_tiles if t[1] == 0][_WO_LAST[-3]:][:n_final]
    last = [(_WO, start + k) for _, _, start, n in whole for k in range(0, n, _PIECE)]
    order = _stream_order([src.shape[0] for src in sources])
    order = [piece for piece in order if piece not in last] + last
    place = {s: i for i, (operand, s) in enumerate(order) if operand == _WO}
    wo_tiles.sort(key=lambda t: max(place[t[2] + k] for k in range(0, t[3], _PIECE)))
    cuts = [len(wo_tiles) - sum(_WO_LAST[i:]) for i in range(len(_WO_LAST) + 1)]
    cuts = list(range(cuts[0] % _WO_GROUP or _WO_GROUP, cuts[0], _WO_GROUP)) + cuts
    wo_groups = [wo_tiles[a:b] for a, b in zip([0] + cuts[:-1], cuts)]
    group_of = {
        start + k: g
        for g, tiles in enumerate(wo_groups, _WO)
        for _, _, start, n in tiles
        for k in range(0, n, _PIECE)
    }
    stream = _Stream(
        [(group_of[s] if operand == _WO else operand, operand, s) for operand, s in order],
        sources, bases, buf, sems,
    )

    def flat(start, n):
        return buf[start:start + n].reshape(n * _SLAB, _LANES)

    def head_group(base, row0, n, g):
        return buf[base + row0:base + row0 + n, g * _HG:(g + 1) * _HG, :].reshape(n * _HG, D)

    per_slab = _SLAB // _TILE_ROWS

    def cache_tile(k0, n, j):
        first = kv0 + k0 // _TILE_ROWS
        tile = slice(j * _TILE_ROWS, (j + 1) * _TILE_ROWS)
        return buf[first:first + n // _TILE_ROWS, tile, :].reshape(n, _LANES)

    def column_tiles(base):
        per_band = hidden_dim // _LANES // per_slab
        for c in range(per_band):
            slabs = [buf[base + i * per_band + c] for i in range(M // _TILE_ROWS)]
            for r in range(0, _SLAB, _TILE_ROWS):
                yield jnp.concatenate([slab[r:r + _TILE_ROWS] for slab in slabs], axis=0)

    def expand(t):
        return flat(expand0 + t * tile_slabs, tile_slabs)

    x_cp = pltpu.make_async_copy(x_hbm, x_v, small_sems.at[0])
    wr_cp = pltpu.make_async_copy(wr_hbm, wr_v, small_sems.at[1])
    stream.advance(8)
    x_cp.start()
    wr_cp.start()
    stream.advance(_QUEUE)

    square = (_LANES, _LANES)
    for t in range(n_expand):
        e = _iota(square, 1) // _HG + t * per_tile == _iota(square, 0)
        first = expand0 + t * tile_slabs
        buf[first:first + tile_slabs] = e.astype(_BF16).reshape(-1, _SLAB, _LANES)
        if t % 4 == 3:
            stream.advance()
    own_head = _iota((rows, _LANES), 1) % _HG == _iota((rows, _LANES), 0) % _HG

    x_cp.wait()
    wr_cp.wait()
    x = _pad_rows(x_v[...].astype(_F32))
    xc = x - jnp.mean(x, axis=-1, keepdims=True)
    xn_lo = (xc / jnp.sqrt(jnp.mean(xc * xc, axis=-1, keepdims=True) + 1e-5)).astype(_BF16)
    xn = xn_lo.astype(_F32)
    wr = wr_v[...].astype(_F32).reshape(1, M)
    route = jax.nn.sigmoid(jnp.sum(xn * wr, axis=-1, keepdims=True))

    for t in range(M // per_tile):
        m0 = t // n_expand * _LANES
        n = min(_LANES, M - m0)
        rep = _dot(xn_lo[:, m0:m0 + n], expand(t % n_expand)[:n])
        rep = jnp.concatenate(
            [jnp.broadcast_to(rep[b:b + 1], (_HG, _LANES)) for b in range(B)], axis=0
        )
        lhs_v[t] = jnp.where(own_head, rep, 0.0).astype(_BF16)
        if t % 3 == 2:
            stream.advance()
    stream.wait(_WQ)
    q = [jnp.zeros((rows, D), _F32) for _ in range(n_groups)]
    for t in range(M // per_tile):
        lhs = lhs_v[t]
        for g in range(n_groups):
            q[g] = q[g] + _dot(lhs, head_group(q0, t * per_tile, per_tile, g))
        if t % 6 == 5:
            stream.advance()

    stream.wait(_WUK)
    q_lat = []
    for g in range(n_groups):
        qg = q[g].astype(_BF16)
        tiles = []
        for c0 in range(0, Dc, _LANES):
            acc = jnp.zeros((rows, _LANES), _F32)
            for t in range(n_expand):
                full = _dot_nt(qg, head_group(uk0, c0 + t * per_tile, per_tile, g))
                acc = acc + _dot_nt(jnp.where(own_head, full, 0.0).astype(_BF16), expand(t))
                if t % 4 == 3:
                    stream.advance()
            tiles.append(acc.astype(_BF16))
        q_lat.append(tiles)

    qk_keys, pv_keys = 512, 1024
    lat_tiles = range(Dc // _LANES)

    def scores(b):
        qb = [
            jnp.concatenate([q_lat[g][j][b * _HG:(b + 1) * _HG] for g in range(n_groups)], axis=0)
            for j in lat_tiles
        ]
        chunks = []
        for k0 in range(b * keys, (b + 1) * keys, qk_keys):
            parts = []
            for j in lat_tiles:
                parts.append(_dot_nt(qb[j], cache_tile(k0, qk_keys, j)))
                if j % 2:
                    stream.advance(_ATTENTION_STEP)
            chunks.append(sum(parts[1:], parts[0]))
        return jnp.concatenate(chunks, axis=1) * (D ** -0.5)

    def attend(b, s):
        p = jnp.exp(s - jnp.max(s, axis=-1, keepdims=True))
        denom = jnp.sum(p, axis=-1, keepdims=True)
        p = p.astype(_BF16)
        acc = [jnp.zeros((heads, _LANES), _F32) for _ in lat_tiles]
        for k0 in range(0, keys, pv_keys):
            for j in lat_tiles:
                v = cache_tile(b * keys + k0, pv_keys, j)
                acc[j] = acc[j] + _dot(p[:, k0:k0 + pv_keys], v)
                stream.advance(_ATTENTION_STEP)
        return [(a / denom).astype(_BF16) for a in acc]

    stream.wait(_CKV)
    lat = []
    s = scores(0)
    for b in range(B):
        ahead = scores(b + 1) if b + 1 < B else None
        lat.append(attend(b, s))
        s = ahead

    stream.wait(_WUV)
    for g in range(n_groups):
        ctx = jnp.zeros((rows, D), _F32)
        for j in lat_tiles:
            lg = jnp.concatenate([lb[j][g * _HG:(g + 1) * _HG] for lb in lat], axis=0)
            for t in range(n_expand):
                lhs = jnp.where(own_head, _dot(lg, expand(t)), 0.0).astype(_BF16)
                ctx = ctx + _dot(lhs, head_group(uv0, j * _LANES + t * per_tile, per_tile, g))
                if t % 8 == 7:
                    stream.advance()
        ctx_v[:, g * _HG:(g + 1) * _HG, :] = ctx.reshape(B, _HG, D)
    for h in range(heads):
        rows_v[h] = _pad_rows(ctx_v[:, h, :], rows_v.shape[1]).astype(_BF16)

    def project(base):
        tiles = []
        for j, w in enumerate(column_tiles(base)):
            tiles.append(_dot(xn_lo, w))
            if j % 6 == 5:
                stream.advance()
        return tiles

    stream.wait(_WG)
    gate = [jax.nn.silu(v) for v in project(g0)]
    stream.wait(_WU)
    hidden = [(a * v).astype(_BF16) for a, v in zip(gate, project(u0))]
    stream.wait(_WD)
    y = jnp.zeros(x.shape, _F32)
    for j, w in enumerate(column_tiles(d0)):
        y = y + _dot_nt(hidden[j], w)
        if j % 3 == 2:
            stream.advance(_DOWN_STEP)
    mixed = jax.nn.silu(xn + (xn * 0.0 + y * route))

    s = [jnp.zeros((x.shape[0], n * _SLAB), _F32) for _, n in lane_tiles]

    def write(tiles, sem):
        cols = slice(tiles[0] * _LANES, min((tiles[-1] + 1) * _LANES, M))
        out = x[:, cols] + jnp.concatenate([s[i] for i in tiles], axis=1) * mixed[:, cols]
        out_v[:, cols] = out.astype(out_v.dtype)[:B]
        copy = pltpu.make_async_copy(out_v.at[:, cols], out_hbm.at[:, cols], small_sems.at[sem])
        copy.start()
        return copy

    for g, tiles in enumerate(wo_groups, _WO):
        if tiles is wo_groups[-2]:
            assert all(i == 0 for rest in wo_groups[-2:] for _, i, _, _ in rest)
            early = write(range(1, len(lane_tiles)), 1)
        stream.wait(g)
        for k, (h, i, start, n) in enumerate(tiles):
            s[i] = s[i] + _dot_nt(rows_v[h][:_TILE_ROWS], flat(o0 + start, n))
            if k % 12 == 11:
                stream.advance()
    write(range(1), 0).wait()
    early.wait()


def _slabs(w):
    r, c = w.shape
    w = w.reshape(r // _TILE_ROWS, _TILE_ROWS, c // _LANES, _LANES)
    return w.transpose(0, 2, 1, 3).reshape(-1, _SLAB, _LANES)


@jax.jit
def pallas_recurrent_scan__compressed_kv_cla__moe_arch_mod__decode_kernel(
    A_x: jax.Array,
    A_c_kv: jax.Array,
    A_w_q: jax.Array,
    A_w_uk: jax.Array,
    A_w_uv: jax.Array,
    A_w_o: jax.Array,
    B_x: jax.Array,
    B_w_r: jax.Array,
    B_w_gate: jax.Array,
    B_w_up: jax.Array,
    B_w_down: jax.Array,
):
    del B_x
    B, Sq, M = A_x.shape
    _, Sk, Dc = A_c_kv.shape
    _, H, D = A_w_q.shape
    assert Sq == 1 and H == _SLAB and D == _LANES

    x = A_x.reshape(B, M)
    streamed = [
        A_w_q,
        A_w_uk,
        _slabs(A_c_kv.reshape(B * Sk, Dc)),
        A_w_uv,
        _slabs(B_w_gate),
        _slabs(B_w_up),
        _slabs(B_w_down.T),
        jnp.transpose(A_w_o, (0, 2, 1)).reshape(-1, _SLAB, _LANES),
    ]
    n_slabs = sum(w.shape[0] for w in streamed) + _HG * _LANES // _SLAB
    n_wo_groups = pl.cdiv(H * pl.cdiv(M, _LANES) - sum(_WO_LAST), _WO_GROUP) + len(_WO_LAST)

    def kernel(*refs):
        _kernel(*refs, heads=H, keys=Sk, hidden_dim=B_w_gate.shape[1])

    hbm = pl.BlockSpec(memory_space=pltpu.HBM)
    out = pl.pallas_call(
        kernel,
        out_shape=jax.ShapeDtypeStruct((B, M), A_x.dtype),
        in_specs=[hbm] * (2 + len(streamed)),
        out_specs=hbm,
        scratch_shapes=[
            pltpu.VMEM((n_slabs, _SLAB, _LANES), _BF16),
            pltpu.VMEM(x.shape, x.dtype),
            pltpu.VMEM(B_w_r.shape, B_w_r.dtype),
            pltpu.VMEM(x.shape, x.dtype),
            pltpu.VMEM((M * _HG // D, B * _HG, D), _BF16),
            pltpu.VMEM((B, H, D), _F32),
            pltpu.VMEM((H, 2 * _TILE_ROWS, D), _BF16),
            pltpu.SemaphoreType.DMA((_WO + n_wo_groups,)),
            pltpu.SemaphoreType.DMA((2,)),
        ],
        compiler_params=pltpu.CompilerParams(
            vmem_limit_bytes=96 * 1024 * 1024, disable_semaphore_checks=True
        ),
    )(x, B_w_r, *streamed)
    return out.reshape(B, Sq, M)
```
